```python
import os as _os
_os.environ.setdefault("JAX_PLATFORMS", "cpu")
import jax
import jax.numpy as jnp

def _softmax(x, axis=-1):
    return jax.nn.softmax(x, axis=axis)
def _gelu(x):
    return jax.nn.gelu(x, approximate=True)
def _silu(x):
    return jax.nn.silu(x)
def _sigmoid(x):
    return jax.nn.sigmoid(x)
def _layernorm(x, axis=-1, eps=1e-5):
    m = jnp.mean(x, axis=axis, keepdims=True)
    v = jnp.var(x, axis=axis, keepdims=True)
    return (x - m) / jnp.sqrt(v + eps)
def _scatter_add(tgt, idx, src, axis=0):
    return tgt.at[idx].add(src)
def _segment_sum(src, seg, n):
    return jax.ops.segment_sum(src, seg, n)
class _Rng:
    def __init__(self, key):
        self._k = key
    def _next(self):
        self._k, sub = jax.random.split(self._k)
        return sub
    def normal(self, shape):
        return jax.random.normal(self._next(), shape, dtype=jnp.bfloat16)
    def randint(self, lo, hi, shape):
        return jax.random.randint(self._next(), shape, lo, hi, dtype=jnp.int32)
    def uniform(self, shape, lo=0.0, hi=1.0):
        return jax.random.uniform(self._next(), shape, jnp.bfloat16, lo, hi)
    def permutation(self, n):
        return jax.random.permutation(self._next(), n)


kernel_name = 'gated_mix__linear_attn_block__glu_gated_swiglu__prompt'

def setup_inputs():
    _rng = _Rng(jax.random.key(int.from_bytes(__import__("os").urandom(4), "little")))
    _w = (lambda a: (lambda t: t.astype(jnp.bfloat16) if jnp.issubdtype(t.dtype, jnp.floating) else t)(jnp.asarray(a)))
    def _A_setup():
        B, S, D = 1, 2048, 1024
        return {
            "x": _w((lambda *s: _rng.normal(s) * 0.05)(B, S, D)),
            "wqkv": _w((lambda *s: _rng.normal(s) * 0.8)(D, 3 * D)),
            "wo": _w((lambda *s: _rng.normal(s) * 0.05)(D, D)),
        }
    _A_in = _A_setup()

    def _B_setup():
        B, S, D, F = 1, 2048, 1024, 3584
        return {
            "x": _w((lambda *s: _rng.normal(s) * 0.05)(B, S, D)),
            "w1": _w((lambda *s: _rng.normal(s) * 1.6)(D, F) * (2.0 / D) ** 0.5),
            "w3": _w((lambda *s: _rng.normal(s) * 1.6)(D, F) * (2.0 / D) ** 0.5),
            "w2": _w((lambda *s: _rng.normal(s) * 1.6)(F, D) * (2.0 / F) ** 0.5),
        }
    _B_in = _B_setup()

    return {
        "A_x": _A_in["x"],
        "A_wqkv": _A_in["wqkv"],
        "A_wo": _A_in["wo"],
        "B_x": _B_in["x"],
        "B_w1": _B_in["w1"],
        "B_w3": _B_in["w3"],
        "B_w2": _B_in["w2"],
        "gate_w": _w((lambda *s: _rng.normal(s) * 0.05)(1024) * 16.0),
    }

def reference(A_x, A_wqkv, A_wo, B_x, B_w1, B_w3, B_w2, gate_w):
    def _A_ref(x, wqkv, wo):
        B, S, D = x.shape
        H = 32; Dh = D // H
        qkv = (lambda x, *d: x.transpose(*d))((x @ wqkv).reshape(B, S, 3, H, Dh), 2, 0, 3, 1, 4)
        q, k, v = qkv[0], qkv[1], qkv[2]
        phi = lambda t: jnp.where(t > 0, t + 1, jnp.exp(t)) + 1e-6
        pq, pk = phi(q), phi(k)
        kv = jnp.einsum("bhsd,bhse->bhde", pk, v)
        z = jnp.einsum("bhsd->bhd", pk)
        num = jnp.einsum("bhqd,bhde->bhqe", pq, kv)
        den = jnp.einsum("bhqd,bhd->bhq", pq, z)[..., None] + 1e-6
        o = num / den
        return (lambda x, *d: x.transpose(*d))(o, 0, 2, 1, 3).reshape(B, S, D) @ wo

    def _B_ref(x, w1, w3, w2):
        gate = jnp.einsum("bsd,df->bsf", x, w1)
        up = jnp.einsum("bsd,df->bsf", x, w3)
        h = _silu(gate) * up
        out = jnp.einsum("bsf,fd->bsd", h, w2)
        return out

    x = A_x
    g = _sigmoid((x * gate_w).sum(-1, keepdims=True))
    a = _A_ref(x, A_wqkv, A_wo)
    b = _B_ref(x, B_w1, B_w3, B_w2)
    return g * a + (1 - g) * b
```

```python
import functools

import jax
import jax.numpy as jnp
import jax.experimental.pallas as pl
import jax.experimental.pallas.tpu as pltpu

H = 32
LG = 128
TM = 256
TF = 3584
WC = 256
FC = 512

def _phi(t):
    return jnp.where(t > 0, t + 1.0, jnp.exp(t)) + 1e-6

def _kernel(x_hbm, gw_ref, wqkv_hbm, wo_hbm, w1_hbm, w3_hbm, w2_hbm, o_ref,
            x_v, wqkv_v, wo_v, w1_v, w3_v, w2_v, kv_acc, z_acc, kvz_b, sems,
            *, S, D, F):
    NT = S // TM
    NF = F // TF
    NFC = F // FC
    NG = D // LG
    NQ = (3 * D) // WC
    Dh = D // H
    step = pl.program_id(0)

    def cp_x(t):
        return pltpu.make_async_copy(
            x_hbm.at[pl.ds(t * TM, TM), :], x_v.at[pl.ds(t * TM, TM), :], sems.at[t])
    B0 = NT
    def cp_qkv(c):
        return pltpu.make_async_copy(
            wqkv_hbm.at[:, pl.ds(c * WC, WC)], wqkv_v.at[:, pl.ds(c * WC, WC)], sems.at[B0 + c])
    def cp_wo():
        return pltpu.make_async_copy(wo_hbm, wo_v, sems.at[B0 + NQ])
    B1 = B0 + NQ + 1
    def cp_w1(c):
        return pltpu.make_async_copy(
            w1_hbm.at[:, pl.ds(c * FC, FC)], w1_v.at[:, pl.ds(c * FC, FC)], sems.at[B1 + c])
    def cp_w3(c):
        return pltpu.make_async_copy(
            w3_hbm.at[:, pl.ds(c * FC, FC)], w3_v.at[:, pl.ds(c * FC, FC)], sems.at[B1 + NFC + c])
    def cp_w2(c):
        return pltpu.make_async_copy(
            w2_hbm.at[pl.ds(c * FC, FC), :], w2_v.at[pl.ds(c * FC, FC), :], sems.at[B1 + 2 * NFC + c])

    nqc = D // WC

    def phase1_body(x, first):
        if first:
            ks = []
            for c in range(nqc):
                cp_qkv(nqc + c).wait()
                ks.append(jnp.dot(x, wqkv_v[:, D + c * WC:D + (c + 1) * WC],
                                  preferred_element_type=jnp.float32))
            k = jnp.concatenate(ks, axis=1)
        else:
            k = jnp.dot(x, wqkv_v[:, D:2 * D], preferred_element_type=jnp.float32)
        pk = _phi(k).astype(jnp.bfloat16)
        if first:
            vs = []
            for c in range(nqc):
                cp_qkv(2 * nqc + c).wait()
                vs.append(jnp.dot(x, wqkv_v[:, 2 * D + c * WC:2 * D + (c + 1) * WC],
                                  preferred_element_type=jnp.float32).astype(jnp.bfloat16))
            v = jnp.concatenate(vs, axis=1)
        else:
            v = jnp.dot(x, wqkv_v[:, 2 * D:3 * D], preferred_element_type=jnp.float32).astype(jnp.bfloat16)
        zs = jnp.sum(pk.astype(jnp.float32).reshape(TM // 8, 8, D), axis=0)
        if first:
            z_acc[...] = zs
        else:
            z_acc[...] += zs
        for g in range(NG):
            pkg = pk[:, g * LG:(g + 1) * LG]
            kvg = jax.lax.dot_general(
                pkg, v[:, g * LG:(g + 1) * LG], (((0,), (0,)), ((), ())),
                preferred_element_type=jnp.float32)
            if first:
                kv_acc[g] = kvg
            else:
                kv_acc[g] += kvg

    @pl.when(step == 0)
    def _start():
        cp_x(0).start()
        for c in range(nqc, 3 * nqc):
            cp_qkv(c).start()
        for t in range(1, NT):
            cp_x(t).start()
        for c in range(nqc):
            cp_qkv(c).start()
        cp_wo().start()
        for c in range(NFC):
            cp_w1(c).start()
            cp_w3(c).start()
        for c in range(NFC):
            cp_w2(c).start()
        cp_x(0).wait()
        phase1_body(x_v[0:TM, :], True)

    @pl.when(jnp.logical_and(step > 0, step < NT))
    def _phase1():
        cp_x(step).wait()
        x = x_v[pl.ds(pl.multiple_of(step * TM, TM), TM), :]
        phase1_body(x, False)

    @pl.when(step >= NT)
    def _phase2():
        @pl.when(step == NT)
        def _():
            r = jax.lax.broadcasted_iota(jnp.int32, (LG, LG), 0)
            c = jax.lax.broadcasted_iota(jnp.int32, (LG, LG), 1)
            mask = (r // Dh) == (c // Dh)
            z = jnp.sum(z_acc[...], axis=0, keepdims=True)
            for g in range(NG):
                zrow = jnp.broadcast_to(z[:, g * LG:(g + 1) * LG], (LG, LG))
                zcol = jnp.transpose(zrow)
                kvz_b[g, :, 0:LG] = jnp.where(mask, kv_acc[g], 0.0).astype(jnp.bfloat16)
                kvz_b[g, :, LG:2 * LG] = jnp.where(mask, zcol, 0.0).astype(jnp.bfloat16)
            for c in range(nqc):
                cp_qkv(c).wait()
            cp_wo().wait()
            for c in range(NFC):
                cp_w1(c).wait()
                cp_w3(c).wait()
                cp_w2(c).wait()

        x = x_v[pl.ds(pl.multiple_of((step - NT) * TM, TM), TM), :]
        q = jnp.dot(x, wqkv_v[:, 0:D], preferred_element_type=jnp.float32)
        pq = _phi(q).astype(jnp.bfloat16)
        os_ = []
        for g in range(NG):
            nd = jnp.dot(pq[:, g * LG:(g + 1) * LG], kvz_b[g], preferred_element_type=jnp.float32)
            os_.append((nd[:, :LG] / (nd[:, LG:] + 1e-6)).astype(jnp.bfloat16))
        o = jnp.concatenate(os_, axis=1)
        a = jnp.dot(o, wo_v[...], preferred_element_type=jnp.float32)

        b = None
        for c in range(NF):
            gate = jnp.dot(x, w1_v[:, c * TF:(c + 1) * TF], preferred_element_type=jnp.float32)
            up = jnp.dot(x, w3_v[:, c * TF:(c + 1) * TF], preferred_element_type=jnp.float32)
            h = (gate * jax.nn.sigmoid(gate) * up).astype(jnp.bfloat16)
            part = jnp.dot(h, w2_v[c * TF:(c + 1) * TF, :], preferred_element_type=jnp.float32)
            b = part if b is None else b + part

        gl = jnp.sum(x.astype(jnp.float32) * gw_ref[...].astype(jnp.float32).reshape(1, D), axis=-1, keepdims=True)
        gt = jax.nn.sigmoid(gl)
        o_ref[...] = (gt * a + (1.0 - gt) * b).astype(o_ref.dtype)


@jax.jit
def pallas_gated_mix__linear_attn_block__glu_gated_swiglu__prompt_kernel(
    A_x, A_wqkv, A_wo, B_x, B_w1, B_w3, B_w2, gate_w):
    B, S, D = A_x.shape
    F = B_w1.shape[1]
    NT = S // TM
    NFC = F // FC
    NG = D // LG
    NQ = (3 * D) // WC
    x2 = A_x.reshape(S, D)
    gw2 = gate_w
    grid_spec = pltpu.PrefetchScalarGridSpec(
        num_scalar_prefetch=0,
        grid=(2 * NT,),
        in_specs=[
            pl.BlockSpec(memory_space=pl.ANY),
            pl.BlockSpec((D,), lambda i: (0,)),
            pl.BlockSpec(memory_space=pl.ANY),
            pl.BlockSpec(memory_space=pl.ANY),
            pl.BlockSpec(memory_space=pl.ANY),
            pl.BlockSpec(memory_space=pl.ANY),
            pl.BlockSpec(memory_space=pl.ANY),
        ],
        out_specs=pl.BlockSpec((TM, D), lambda i: (jnp.maximum(i - NT, 0), 0)),
        scratch_shapes=[
            pltpu.VMEM((S, D), jnp.bfloat16),
            pltpu.VMEM((D, 3 * D), jnp.bfloat16),
            pltpu.VMEM((D, D), jnp.bfloat16),
            pltpu.VMEM((D, F), jnp.bfloat16),
            pltpu.VMEM((D, F), jnp.bfloat16),
            pltpu.VMEM((F, D), jnp.bfloat16),
            pltpu.VMEM((NG, LG, LG), jnp.float32),
            pltpu.VMEM((8, D), jnp.float32),
            pltpu.VMEM((NG, LG, 2 * LG), jnp.bfloat16),
            pltpu.SemaphoreType.DMA((NT + NQ + 1 + 3 * NFC,)),
        ],
    )
    out = pl.pallas_call(
        functools.partial(_kernel, S=S, D=D, F=F),
        grid_spec=grid_spec,
        out_shape=jax.ShapeDtypeStruct((S, D), A_x.dtype),
        compiler_params=pltpu.CompilerParams(
            dimension_semantics=("arbitrary",),
            vmem_limit_bytes=110 * 1024 * 1024,
        ),
    )(x2, gw2, A_wqkv, A_wo, B_w1, B_w3, B_w2)
    return out.reshape(B, S, D)
```

```python
import functools

import jax
import jax.numpy as jnp
import jax.experimental.pallas as pl
import jax.experimental.pallas.tpu as pltpu

H = 32
LG = 128
TM = 256
WC = 256
FC = 512


def _phi(t):
    return jnp.where(t > 0, t + 1.0, jnp.exp(t)) + 1e-6


def _kernel(x_hbm, gw_ref, wqkv_hbm, wo_hbm, w1_hbm, w3_hbm, w2_hbm, o_ref,
            x_v, wqkv_v, wo_v, w1_v, w3_v, w2_v, kv_acc, z_acc, kvz_b, kv0_s, sems,
            *, S, D, F):
    NT = S // TM
    NFC = F // FC
    NG = D // LG
    NQ = (3 * D) // WC
    nqc = D // WC
    Dh = D // H
    step = pl.program_id(0)

    B0 = NT
    B1 = B0 + NQ + 1

    def cp_x(t):
        return pltpu.make_async_copy(
            x_hbm.at[pl.ds(t * TM, TM), :], x_v.at[pl.ds(t * TM, TM), :], sems.at[t])

    def cp_qkv(c):
        return pltpu.make_async_copy(
            wqkv_hbm.at[:, pl.ds(c * WC, WC)], wqkv_v.at[:, pl.ds(c * WC, WC)],
            sems.at[B0 + c])

    def cp_wo():
        return pltpu.make_async_copy(wo_hbm, wo_v, sems.at[B0 + NQ])

    def cp_w1(c):
        return pltpu.make_async_copy(
            w1_hbm.at[:, pl.ds(c * FC, FC)], w1_v.at[:, pl.ds(c * FC, FC)],
            sems.at[B1 + c])

    def cp_w3(c):
        return pltpu.make_async_copy(
            w3_hbm.at[:, pl.ds(c * FC, FC)], w3_v.at[:, pl.ds(c * FC, FC)],
            sems.at[B1 + NFC + c])

    def cp_w2(c):
        return pltpu.make_async_copy(
            w2_hbm.at[pl.ds(c * FC, FC), :], w2_v.at[pl.ds(c * FC, FC), :],
            sems.at[B1 + 2 * NFC + c])

    def phase1_post(k, v, first):
        pk = _phi(k).astype(jnp.bfloat16)
        zs = jnp.sum(pk.astype(jnp.float32).reshape(TM // 8, 8, D), axis=0)
        if first:
            z_acc[...] = zs
        else:
            z_acc[...] += zs
        for g in range(NG):
            kvg = jax.lax.dot_general(
                pk[:, g * LG:(g + 1) * LG], v[:, g * LG:(g + 1) * LG],
                (((0,), (0,)), ((), ())), preferred_element_type=jnp.float32)
            if first:
                kv_acc[g] = kvg
            else:
                kv_acc[g] += kvg

    @pl.when(step == 0)
    def _step0():
        cp_x(0).start()
        for c in range(nqc, 3 * nqc):
            cp_qkv(c).start()
        for t in range(1, NT):
            cp_x(t).start()
        for c in range(nqc):
            cp_qkv(c).start()
        cp_wo().start()
        for c in range(NFC):
            cp_w1(c).start()
            cp_w3(c).start()
        for c in range(NFC):
            cp_w2(c).start()
        cp_x(0).wait()

        def chunk(c, carry):
            cp_qkv(nqc + c).wait()
            kv0_s[:, pl.ds(pl.multiple_of(c * WC, WC), WC)] = jnp.dot(
                x_v[0:TM, :], wqkv_v[:, pl.ds(pl.multiple_of(D + c * WC, WC), WC)],
                preferred_element_type=jnp.float32)
            return carry

        jax.lax.fori_loop(0, 2 * nqc, chunk, 0)
        phase1_post(kv0_s[:, 0:D], kv0_s[:, D:2 * D].astype(jnp.bfloat16), True)

    @pl.when(jnp.logical_and(step > 0, step < NT))
    def _phase1():
        cp_x(step).wait()
        x = x_v[pl.ds(pl.multiple_of(step * TM, TM), TM), :]
        k = jnp.dot(x, wqkv_v[:, D:2 * D], preferred_element_type=jnp.float32)
        v = jnp.dot(x, wqkv_v[:, 2 * D:3 * D],
                    preferred_element_type=jnp.float32).astype(jnp.bfloat16)
        phase1_post(k, v, False)

    @pl.when(step >= NT)
    def _phase2():
        @pl.when(step == NT)
        def _transition():
            r = jax.lax.broadcasted_iota(jnp.int32, (LG, LG), 0)
            c = jax.lax.broadcasted_iota(jnp.int32, (LG, LG), 1)
            mask = (r // Dh) == (c // Dh)
            z = jnp.sum(z_acc[...], axis=0, keepdims=True)
            for g in range(NG):
                zrow = jnp.broadcast_to(z[:, g * LG:(g + 1) * LG], (LG, LG))
                zcol = jnp.transpose(zrow)
                kvz_b[g, :, 0:LG] = jnp.where(mask, kv_acc[g], 0.0).astype(jnp.bfloat16)
                kvz_b[g, :, LG:2 * LG] = jnp.where(mask, zcol, 0.0).astype(jnp.bfloat16)
            for c in range(nqc):
                cp_qkv(c).wait()
            cp_wo().wait()
            for c in range(NFC):
                cp_w1(c).wait()
                cp_w3(c).wait()
                cp_w2(c).wait()

        x = x_v[pl.ds(pl.multiple_of((step - NT) * TM, TM), TM), :]

        q = jnp.dot(x, wqkv_v[:, 0:D], preferred_element_type=jnp.float32)
        pq = _phi(q).astype(jnp.bfloat16)
        os_ = []
        for g in range(NG):
            nd = jnp.dot(pq[:, g * LG:(g + 1) * LG], kvz_b[g],
                         preferred_element_type=jnp.float32)
            os_.append((nd[:, :LG] / (nd[:, LG:] + 1e-6)).astype(jnp.bfloat16))
        o = jnp.concatenate(os_, axis=1)
        a = jnp.dot(o, wo_v[...], preferred_element_type=jnp.float32)

        gate = jnp.dot(x, w1_v[...], preferred_element_type=jnp.float32)
        up = jnp.dot(x, w3_v[...], preferred_element_type=jnp.float32)
        h = (gate * jax.nn.sigmoid(gate) * up).astype(jnp.bfloat16)
        b = jnp.dot(h, w2_v[...], preferred_element_type=jnp.float32)

        gw = gw_ref[...].astype(jnp.float32).reshape(1, D)
        gl = jnp.sum(x.astype(jnp.float32) * gw, axis=-1, keepdims=True)
        gt = jax.nn.sigmoid(gl)
        o_ref[...] = (gt * a + (1.0 - gt) * b).astype(o_ref.dtype)


@jax.jit
def pallas_gated_mix__linear_attn_block__glu_gated_swiglu__prompt_kernel(
    A_x: jax.Array,
    A_wqkv: jax.Array,
    A_wo: jax.Array,
    B_x: jax.Array,
    B_w1: jax.Array,
    B_w3: jax.Array,
    B_w2: jax.Array,
    gate_w: jax.Array,
):
    B, S, D = A_x.shape
    F = B_w1.shape[1]
    assert B == 1 and S % TM == 0 and D % WC == 0 and F % FC == 0 and D % LG == 0
    NT = S // TM
    NFC = F // FC
    NG = D // LG
    NQ = (3 * D) // WC
    x2 = A_x.reshape(S, D)

    grid_spec = pltpu.PrefetchScalarGridSpec(
        num_scalar_prefetch=0,
        grid=(2 * NT,),
        in_specs=[
            pl.BlockSpec(memory_space=pl.ANY),
            pl.BlockSpec((D,), lambda i: (0,)),
            pl.BlockSpec(memory_space=pl.ANY),
            pl.BlockSpec(memory_space=pl.ANY),
            pl.BlockSpec(memory_space=pl.ANY),
            pl.BlockSpec(memory_space=pl.ANY),
            pl.BlockSpec(memory_space=pl.ANY),
        ],
        out_specs=pl.BlockSpec((TM, D), lambda i: (jnp.maximum(i - NT, 0), 0)),
        scratch_shapes=[
            pltpu.VMEM((S, D), jnp.bfloat16),
            pltpu.VMEM((D, 3 * D), jnp.bfloat16),
            pltpu.VMEM((D, D), jnp.bfloat16),
            pltpu.VMEM((D, F), jnp.bfloat16),
            pltpu.VMEM((D, F), jnp.bfloat16),
            pltpu.VMEM((F, D), jnp.bfloat16),
            pltpu.VMEM((NG, LG, LG), jnp.float32),
            pltpu.VMEM((8, D), jnp.float32),
            pltpu.VMEM((NG, LG, 2 * LG), jnp.bfloat16),
            pltpu.VMEM((TM, 2 * D), jnp.float32),
            pltpu.SemaphoreType.DMA((NT + NQ + 1 + 3 * NFC,)),
        ],
    )
    out = pl.pallas_call(
        functools.partial(_kernel, S=S, D=D, F=F),
        grid_spec=grid_spec,
        out_shape=jax.ShapeDtypeStruct((S, D), A_x.dtype),
        compiler_params=pltpu.CompilerParams(
            dimension_semantics=("arbitrary",),
            vmem_limit_bytes=110 * 1024 * 1024,
        ),
    )(x2, gate_w, A_wqkv, A_wo, B_w1, B_w3, B_w2)
    return out.reshape(B, S, D)
```

```python
import functools

import jax
import jax.numpy as jnp
import jax.experimental.pallas as pl
import jax.experimental.pallas.tpu as pltpu

H = 32
LG = 128
TM = 256
WC = 256
FC = 512


def _phi(t):
    return jnp.where(t > 0, t + 1.0, jnp.exp(t)) + 1e-6


def _kernel(x_hbm, gw_ref, wqkv_hbm, wo_hbm, w1_hbm, w3_hbm, w2_hbm, o_ref,
            x_v, wqkv_v, wo_v, w1_v, w3_v, w2_v, kv_acc, z_acc, kvz_b, kv0_s, sems,
            *, S, D, F):
    NT = S // TM
    NFC = F // FC
    NG = D // LG
    NQ = (3 * D) // WC
    nqc = D // WC
    NKV = NQ - nqc
    RC = D // NKV
    Dh = D // H
    step = pl.program_id(0)

    B0 = NT
    B1 = B0 + NQ + 1

    def cp_x(t):
        return pltpu.make_async_copy(
            x_hbm.at[pl.ds(t * TM, TM), :], x_v.at[pl.ds(t * TM, TM), :], sems.at[t])

    def cp_q(c):
        return pltpu.make_async_copy(
            wqkv_hbm.at[:, pl.ds(c * WC, WC)], wqkv_v.at[:, pl.ds(c * WC, WC)],
            sems.at[B0 + c])

    def cp_kv(c):
        return pltpu.make_async_copy(
            wqkv_hbm.at[pl.ds(c * RC, RC), pl.ds(D, 2 * D)],
            wqkv_v.at[pl.ds(c * RC, RC), pl.ds(D, 2 * D)],
            sems.at[B0 + nqc + c])

    def cp_wo():
        return pltpu.make_async_copy(wo_hbm, wo_v, sems.at[B0 + NQ])

    def cp_w1(c):
        return pltpu.make_async_copy(
            w1_hbm.at[:, pl.ds(c * FC, FC)], w1_v.at[:, pl.ds(c * FC, FC)],
            sems.at[B1 + c])

    def cp_w3(c):
        return pltpu.make_async_copy(
            w3_hbm.at[:, pl.ds(c * FC, FC)], w3_v.at[:, pl.ds(c * FC, FC)],
            sems.at[B1 + NFC + c])

    def cp_w2(c):
        return pltpu.make_async_copy(
            w2_hbm.at[pl.ds(c * FC, FC), :], w2_v.at[pl.ds(c * FC, FC), :],
            sems.at[B1 + 2 * NFC + c])

    def phase1_post(k, v, first):
        pk = _phi(k).astype(jnp.bfloat16)
        zs = jnp.sum(pk.astype(jnp.float32).reshape(TM // 8, 8, D), axis=0)
        if first:
            z_acc[...] = zs
        else:
            z_acc[...] += zs
        for g in range(NG):
            kvg = jax.lax.dot_general(
                pk[:, g * LG:(g + 1) * LG], v[:, g * LG:(g + 1) * LG],
                (((0,), (0,)), ((), ())), preferred_element_type=jnp.float32)
            if first:
                kv_acc[g] = kvg
            else:
                kv_acc[g] += kvg

    @pl.when(step == 0)
    def _step0():
        cp_x(0).start()
        for c in range(NKV):
            cp_kv(c).start()
        for t in range(1, NT):
            cp_x(t).start()
        for c in range(nqc):
            cp_q(c).start()
        cp_wo().start()
        for c in range(NFC):
            cp_w1(c).start()
            cp_w3(c).start()
        for c in range(NFC):
            cp_w2(c).start()
        cp_x(0).wait()

        cp_kv(0).wait()
        kv0_s[...] = jnp.dot(x_v[0:TM, 0:RC], wqkv_v[0:RC, D:3 * D],
                             preferred_element_type=jnp.float32)

        def chunk(c, carry):
            cp_kv(c).wait()
            off = pl.multiple_of(c * RC, RC)
            kv0_s[...] += jnp.dot(
                x_v[0:TM, pl.ds(off, RC)], wqkv_v[pl.ds(off, RC), D:3 * D],
                preferred_element_type=jnp.float32)
            return carry

        jax.lax.fori_loop(1, NKV, chunk, 0)
        phase1_post(kv0_s[:, 0:D], kv0_s[:, D:2 * D].astype(jnp.bfloat16), True)

    @pl.when(jnp.logical_and(step > 0, step < NT))
    def _phase1():
        cp_x(step).wait()
        x = x_v[pl.ds(pl.multiple_of(step * TM, TM), TM), :]
        k = jnp.dot(x, wqkv_v[:, D:2 * D], preferred_element_type=jnp.float32)
        v = jnp.dot(x, wqkv_v[:, 2 * D:3 * D],
                    preferred_element_type=jnp.float32).astype(jnp.bfloat16)
        phase1_post(k, v, False)

    @pl.when(step >= NT)
    def _phase2():
        @pl.when(step == NT)
        def _transition():
            r = jax.lax.broadcasted_iota(jnp.int32, (LG, LG), 0)
            c = jax.lax.broadcasted_iota(jnp.int32, (LG, LG), 1)
            mask = (r // Dh) == (c // Dh)
            z = jnp.sum(z_acc[...], axis=0, keepdims=True)
            for g in range(NG):
                zrow = jnp.broadcast_to(z[:, g * LG:(g + 1) * LG], (LG, LG))
                zcol = jnp.transpose(zrow)
                kvz_b[g, :, 0:LG] = jnp.where(mask, kv_acc[g], 0.0).astype(jnp.bfloat16)
                kvz_b[g, :, LG:2 * LG] = jnp.where(mask, zcol, 0.0).astype(jnp.bfloat16)
            for c in range(nqc):
                cp_q(c).wait()
            cp_wo().wait()
            for c in range(NFC):
                cp_w1(c).wait()
                cp_w3(c).wait()
                cp_w2(c).wait()

        x = x_v[pl.ds(pl.multiple_of((step - NT) * TM, TM), TM), :]

        q = jnp.dot(x, wqkv_v[:, 0:D], preferred_element_type=jnp.float32)
        pq = _phi(q).astype(jnp.bfloat16)
        os_ = []
        for g in range(NG):
            nd = jnp.dot(pq[:, g * LG:(g + 1) * LG], kvz_b[g],
                         preferred_element_type=jnp.float32)
            os_.append((nd[:, :LG] / (nd[:, LG:] + 1e-6)).astype(jnp.bfloat16))
        o = jnp.concatenate(os_, axis=1)
        a = jnp.dot(o, wo_v[...], preferred_element_type=jnp.float32)

        gate = jnp.dot(x, w1_v[...], preferred_element_type=jnp.float32)
        up = jnp.dot(x, w3_v[...], preferred_element_type=jnp.float32)
        h = (gate * jax.nn.sigmoid(gate) * up).astype(jnp.bfloat16)
        b = jnp.dot(h, w2_v[...], preferred_element_type=jnp.float32)

        gw = gw_ref[...].astype(jnp.float32).reshape(1, D)
        gl = jnp.sum(x.astype(jnp.float32) * gw, axis=-1, keepdims=True)
        gt = jax.nn.sigmoid(gl)
        o_ref[...] = (gt * a + (1.0 - gt) * b).astype(o_ref.dtype)


@jax.jit
def pallas_gated_mix__linear_attn_block__glu_gated_swiglu__prompt_kernel(
    A_x: jax.Array,
    A_wqkv: jax.Array,
    A_wo: jax.Array,
    B_x: jax.Array,
    B_w1: jax.Array,
    B_w3: jax.Array,
    B_w2: jax.Array,
    gate_w: jax.Array,
):
    B, S, D = A_x.shape
    F = B_w1.shape[1]
    assert B == 1 and S % TM == 0 and D % WC == 0 and F % FC == 0 and D % LG == 0
    NT = S // TM
    NFC = F // FC
    NG = D // LG
    NQ = (3 * D) // WC
    x2 = A_x.reshape(S, D)

    grid_spec = pltpu.PrefetchScalarGridSpec(
        num_scalar_prefetch=0,
        grid=(2 * NT,),
        in_specs=[
            pl.BlockSpec(memory_space=pl.ANY),
            pl.BlockSpec((D,), lambda i: (0,)),
            pl.BlockSpec(memory_space=pl.ANY),
            pl.BlockSpec(memory_space=pl.ANY),
            pl.BlockSpec(memory_space=pl.ANY),
            pl.BlockSpec(memory_space=pl.ANY),
            pl.BlockSpec(memory_space=pl.ANY),
        ],
        out_specs=pl.BlockSpec((TM, D), lambda i: (jnp.maximum(i - NT, 0), 0)),
        scratch_shapes=[
            pltpu.VMEM((S, D), jnp.bfloat16),
            pltpu.VMEM((D, 3 * D), jnp.bfloat16),
            pltpu.VMEM((D, D), jnp.bfloat16),
            pltpu.VMEM((D, F), jnp.bfloat16),
            pltpu.VMEM((D, F), jnp.bfloat16),
            pltpu.VMEM((F, D), jnp.bfloat16),
            pltpu.VMEM((NG, LG, LG), jnp.float32),
            pltpu.VMEM((8, D), jnp.float32),
            pltpu.VMEM((NG, LG, 2 * LG), jnp.bfloat16),
            pltpu.VMEM((TM, 2 * D), jnp.float32),
            pltpu.SemaphoreType.DMA((NT + NQ + 1 + 3 * NFC,)),
        ],
    )
    out = pl.pallas_call(
        functools.partial(_kernel, S=S, D=D, F=F),
        grid_spec=grid_spec,
        out_shape=jax.ShapeDtypeStruct((S, D), A_x.dtype),
        compiler_params=pltpu.CompilerParams(
            dimension_semantics=("arbitrary",),
            vmem_limit_bytes=110 * 1024 * 1024,
        ),
    )(x2, gate_w, A_wqkv, A_wo, B_w1, B_w3, B_w2)
    return out.reshape(B, S, D)
```
